```python
import os as _os
_os.environ.setdefault("JAX_PLATFORMS", "cpu")
import jax
import jax.numpy as jnp

def _softmax(x, axis=-1):
    return jax.nn.softmax(x, axis=axis)
def _gelu(x):
    return jax.nn.gelu(x, approximate=True)
def _silu(x):
    return jax.nn.silu(x)
def _sigmoid(x):
    return jax.nn.sigmoid(x)
def _layernorm(x, axis=-1, eps=1e-5):
    m = jnp.mean(x, axis=axis, keepdims=True)
    v = jnp.var(x, axis=axis, keepdims=True)
    return (x - m) / jnp.sqrt(v + eps)
def _scatter_add(tgt, idx, src, axis=0):
    return tgt.at[idx].add(src)
def _segment_sum(src, seg, n):
    return jax.ops.segment_sum(src, seg, n)
class _Rng:
    def __init__(self, key):
        self._k = key
    def _next(self):
        self._k, sub = jax.random.split(self._k)
        return sub
    def normal(self, shape):
        return jax.random.normal(self._next(), shape, dtype=jnp.bfloat16)
    def randint(self, lo, hi, shape):
        return jax.random.randint(self._next(), shape, lo, hi, dtype=jnp.int32)
    def uniform(self, shape, lo=0.0, hi=1.0):
        return jax.random.uniform(self._next(), shape, jnp.bfloat16, lo, hi)
    def permutation(self, n):
        return jax.random.permutation(self._next(), n)


kernel_name = 'parallel_sum__grouped_kv_mqa__dense_activation_silu__prompt'

def setup_inputs():
    _rng = _Rng(jax.random.key(int.from_bytes(__import__("os").urandom(4), "little")))
    _w = (lambda a: (lambda t: t.astype(jnp.bfloat16) if jnp.issubdtype(t.dtype, jnp.floating) else t)(jnp.asarray(a)))
    def _A_setup():
        B, S, D, H = 1, 2048, 512, 32
        Dh = D // H
        return {
            "x": _w((lambda *s: _rng.normal(s) * 0.05)(B, S, D)),
            "wq": _w((lambda *s: _rng.normal(s) * 0.05)(D, H * Dh)),
            "wk": _w((lambda *s: _rng.normal(s) * 0.05)(D, Dh)),
            "wv": _w((lambda *s: _rng.normal(s) * 0.05)(D, Dh)),
            "wo": _w((lambda *s: _rng.normal(s) * 0.05)(H * Dh, D)),
        }
    _A_in = _A_setup()

    def _B_setup():
        B, S, D, F = 1, 2048, 512, 1792
        return {
            "x": _w((lambda *s: _rng.normal(s) * 0.05)(B, S, D)),
            "w1": _w((lambda *s: _rng.normal(s) * 0.05)(D, F) * (D ** -0.5)),
            "w2": _w((lambda *s: _rng.normal(s) * 0.05)(F, D) * (F ** -0.5)),
        }
    _B_in = _B_setup()

    return {
        "A_x": _A_in["x"],
        "A_wq": _A_in["wq"],
        "A_wk": _A_in["wk"],
        "A_wv": _A_in["wv"],
        "A_wo": _A_in["wo"],
        "B_x": _B_in["x"],
        "B_w1": _B_in["w1"],
        "B_w2": _B_in["w2"],
    }

def reference(A_x, A_wq, A_wk, A_wv, A_wo, B_x, B_w1, B_w2):
    def _A_ref(x, wq, wk, wv, wo):
        B, S, D = x.shape
        H = 32
        Dh = D // H
        q = (lambda x, *d: x.transpose(*d))((x @ wq).reshape(B, S, H, Dh), 0, 2, 1, 3)
        k = x @ wk
        v = x @ wv
        scores = jnp.einsum("bhqd,bkd->bhqk", q, k) * (Dh ** -0.5)
        p = _softmax(scores, axis=-1)
        o = jnp.einsum("bhqk,bkd->bhqd", p, v)
        return (lambda x, *d: x.transpose(*d))(o, 0, 2, 1, 3).reshape(B, S, H * Dh) @ wo

    def _B_ref(x, w1, w2):
        h = jnp.einsum("bsd,df->bsf", x, w1)
        h = _silu(h)
        out = jnp.einsum("bsf,fd->bsd", h, w2)
        return out

    x = A_x
    xn = _layernorm(x, axis=-1)
    return x + _A_ref(xn, A_wq, A_wk, A_wv, A_wo) + _B_ref(xn, B_w1, B_w2)
```

```python
import functools, math
import jax, jax.numpy as jnp
from jax import lax
from jax.experimental import pallas as pl
from jax.experimental.pallas import tpu as pltpu

H = 32
DH = 16
LOG2E = 1.4426950408889634
TQ = 128
GH = 4
NG = H // GH
W = GH * TQ
KD = 96
ALPHA = 16.0
BETA = 16.0
BOUND = 48.0
f32 = jnp.float32
bf16 = jnp.bfloat16
NT = (((1,), (1,)), ((), ()))
TN = (((0,), (0,)), ((), ()))


def _rint(x):
    return jnp.round(x).astype(jnp.int32)


def _rev16(a, t):
    return jnp.concatenate([a[t * 128 + (7 - b) * 16: t * 128 + (8 - b) * 16] for b in range(8)], axis=0)


def _kernel(x_hbm, wq_hbm, wkT_ref, wvT_ref, wo_hbm, w1_hbm, w2_hbm, o_ref,
            x_ref, wq_ref, wo_ref, w1_ref, w2_ref, sems,
            xn_ref, wT_ref, kvT_ref, k8_ref, vT_ref, ck_ref, cv_ref, qT_ref, q8_ref, sq_ref, qs_ref, oT_ref, h_ref, acc_ref,
            flag_ref, *, S, D, F, pat, ntail, LC, wstart):
    i = pl.program_id(0)
    nblk = S // TQ
    NCH = S // LC

    def qscale(blk):
        q3 = jnp.abs(qT_ref[blk]).reshape(H, DH, TQ)
        am = jnp.max(q3, axis=0) * ck_ref[...]
        am = jnp.max(am, axis=0, keepdims=True)
        am = jnp.where(am > 0, am, 1.0)
        qs_ref[...] = ck_ref[...] * (254.0 / am)
        return jnp.broadcast_to(am * (1.0 / (254.0 * 254.0)), (8, TQ))

    def quant(blk, g):
        q2 = qT_ref[blk, g * GH * DH:(g + 1) * GH * DH, :].reshape(GH, DH, TQ) * qs_ref[...][None]
        q2i = _rint(q2)
        q2f = q2i.astype(f32)
        qa = q2i >> 1
        qb = q2i - qa
        dq = _rint((q2 - q2f) * ALPHA)
        rq = _rint(q2f * (1.0 / BETA))
        main = jnp.concatenate([qa, qb], axis=1).astype(jnp.int8)
        corr = jnp.concatenate([dq, rq], axis=1).astype(jnp.int8)
        for u in range(GH):
            q8_ref[g, 0:32, u * TQ:(u + 1) * TQ] = main[u]
            q8_ref[g, 32:64, u * TQ:(u + 1) * TQ] = corr[u]

    @pl.when(i == 0)
    def _():
        xcp = [pltpu.make_async_copy(x_hbm.at[pl.ds(c * LC, LC)], x_ref.at[pl.ds(c * LC, LC)], sems.at[c])
               for c in range(NCH)]
        wqcp = pltpu.make_async_copy(wq_hbm, wq_ref, sems.at[NCH])
        wcp = [pltpu.make_async_copy(s_, d_, sems.at[NCH + 1 + n])
               for n, (s_, d_) in enumerate(((w1_hbm, w1_ref), (w2_hbm, w2_ref), (wo_hbm, wo_ref)))]
        xcp[0].start()
        wqcp.start()
        for c in range(1, NCH):
            xcp[c].start()

        def ln(c):
            x = x_ref[c * LC:(c + 1) * LC, :].astype(f32)
            m = jnp.mean(x, axis=-1, keepdims=True)
            xc = x - m
            v = jnp.mean(xc * xc, axis=-1, keepdims=True)
            xn_ref[c * LC:(c + 1) * LC, :] = (xc * lax.rsqrt(v + 1e-5)).astype(bf16)

        def proj(c, qn):
            y = lax.dot_general(wT_ref[...], xn_ref[c * LC:(c + 1) * LC, :], NT, preferred_element_type=f32)
            kvT_ref[:, c * LC:(c + 1) * LC] = y[D:D + 2 * DH]
            for t in range(LC // TQ):
                qT = y[0:D, t * TQ:(t + 1) * TQ] * (DH ** -0.5 * LOG2E)
                qT_ref[c * (LC // TQ) + t] = qT
                q2 = jnp.sum((qT * qT).reshape(H, DH, TQ), axis=1)
                qn = q2 if qn is None else jnp.maximum(qn, q2)
            return qn

        xcp[0].wait()
        ln(0)
        wqcp.wait()
        wT_ref[0:D, :] = wq_ref[...].T
        wT_ref[D:D + DH, :] = wkT_ref[...]
        wT_ref[D + DH:D + 2 * DH, :] = wvT_ref[...]
        qn = None
        for c in range(NCH):
            if c == wstart:
                for cp in wcp:
                    cp.start()
            if c + 1 < NCH:
                xcp[c + 1].wait()
            qn = proj(c, qn)
            if c + 1 < NCH:
                ln(c + 1)

        kvT = kvT_ref[...]
        cmax = jnp.max(jnp.abs(kvT), axis=1, keepdims=True)
        cmax = jnp.where(cmax > 0, cmax, 1.0)
        cb = jnp.broadcast_to(cmax, (2 * DH, 128))
        ck_ref[...] = cb[0:DH]
        cv_ref[...] = cb[DH:2 * DH]
        kvn = kvT * (1.0 / cmax)
        vT_ref[...] = kvn[DH:2 * DH].astype(bf16)
        kT = kvT[0:DH]
        kn2 = jnp.sum(kT * kT, axis=0, keepdims=True)
        flag_ref[0] = (jnp.max(qn) * jnp.max(kn2) <= BOUND * BOUND).astype(jnp.int32)
        k2 = kvn[0:DH] * 254.0
        k2i = _rint(k2)
        ka = k2i >> 1
        kb = k2i - ka
        dk = _rint((k2 - k2i.astype(f32)) * BETA)
        rk = _rint(k2 * (1.0 / ALPHA))
        ka, kb, dk, rk = [a.astype(f32).astype(bf16) for a in (ka, kb, dk, rk)]
        zz = jnp.zeros_like(ka)
        aT = jnp.concatenate([ka, kb, kb, ka, rk, dk, zz, zz], axis=0)
        r = lax.broadcasted_iota(jnp.int32, (128, 128), 0)
        c_ = lax.broadcasted_iota(jnp.int32, (128, 128), 1)
        perm = jnp.where(c_ == (7 - r // 16) * 16 + r % 16, 1.0, 0.0).astype(bf16)
        for t in range(S // 128):
            kt = lax.dot_general(perm, aT[:, t * 128:(t + 1) * 128], NT, preferred_element_type=f32)
            k8_ref[t * 128:(t + 1) * 128, :] = kt.astype(jnp.int32).astype(jnp.int8)
        sq_ref[...] = qscale(0)
        for g in range(NG):
            quant(0, g)
        for cp in wcp:
            cp.wait()

    r0 = pl.multiple_of(i * TQ, TQ)
    nxt = jnp.minimum(i + 1, nblk - 1)
    fast = flag_ref[0] > 0
    NF = F // 128

    def ffn1(c):
        hh = jnp.dot(xn_ref[pl.ds(r0, TQ), :], w1_ref[:, c * 128:(c + 1) * 128], preferred_element_type=f32)
        u = 0.5 * hh
        h_ref[:, c * 128:(c + 1) * 128] = (u + u * jnp.tanh(u)).astype(bf16)

    def ffn2(c):
        y = jnp.dot(h_ref[:, c * 128:(c + 1) * 128], w2_ref[c * 128:(c + 1) * 128, :], preferred_element_type=f32)
        if c == 0:
            acc_ref[...] = y + x_ref[pl.ds(r0, TQ), :].astype(f32)
        else:
            acc_ref[...] += y

    def oproj(n):
        o = oT_ref[n * 128:(n + 1) * 128, :].T.astype(bf16)
        y = jnp.dot(o, wo_ref[n * 128:(n + 1) * 128, :], preferred_element_type=f32)
        if n == 3:
            o_ref[...] = (acc_ref[...] + y).astype(o_ref.dtype)
        else:
            acc_ref[...] += y

    ffn = []
    for c in range(NF):
        ffn.append(functools.partial(ffn1, c))
        if c >= 1:
            ffn.append(functools.partial(ffn2, c - 1))
    ffn.append(functools.partial(ffn2, NF - 1))

    @pl.when(fast)
    def _():
        NT_ = S // 128
        pt = {}
        st = {}
        ls = {}
        sq1 = sq_ref[...]
        sq = jnp.concatenate([sq1] * GH, axis=1)
        sq_next = qscale(nxt)

        def qk(g, t0, nt):
            q8 = q8_ref[g]
            wgt = jnp.concatenate([q8[0:32], q8[0:32], q8[32:64]], axis=0)
            s = jnp.dot(k8_ref[t0 * 128:(t0 + nt) * 128, 0:KD], wgt, preferred_element_type=jnp.int32)
            s = s.astype(f32).reshape(nt * 16, 8, W) * sq[None]
            p = jnp.exp2(s)
            l = jnp.sum(p, axis=0)
            ls[g] = l if t0 == 0 else ls[g] + l
            p = p.reshape(nt * 128, W)
            for t in range(nt):
                pt[(g, t0 + t)] = _rev16(p, t).astype(bf16)

        def pv(g, t):
            o = jnp.dot(vT_ref[:, t * 128:(t + 1) * 128], pt.pop((g, t)), preferred_element_type=f32)
            st[g] = o if t == 0 else st[g] + o
            if t == NT_ - 1:
                res = st.pop(g) * (1.0 / jnp.sum(ls.pop(g), axis=0, keepdims=True))
                for u in range(GH):
                    h = g * GH + u
                    oT_ref[h * DH:(h + 1) * DH, :] = res[:, u * TQ:(u + 1) * TQ] * cv_ref[...]

        dense = list(ffn)
        tail = [dense.pop() for _ in range(ntail)][::-1]
        nit = NG * NT_ // 2
        nd = len(dense) + 3
        pos = [int(round(j * (nit - 1) / (nd - 1))) for j in range(nd)]
        opos = {}
        for n in range(3):
            first = (2 * n + 2) * 8 + 2
            pidx = min(k for k, p_ in enumerate(pos) if p_ >= first and k not in opos.values())
            opos[n] = pidx
        sched = {}
        for k, p_ in enumerate(pos):
            o = [n for n, v in opos.items() if v == k]
            d = functools.partial(oproj, o[0]) if o else dense.pop(0)
            sched.setdefault(p_, []).append(d)
        assert not dense
        for j in range(nit + 1):
            if j >= 8 and j % 8 == 0:
                quant(nxt, j // 8 - 1)
            if j < nit:
                g, t0 = divmod(j * 2, NT_)
                qk(g, t0, 2)
            if pat == 3:
                for d in sched.get(j, []): d()
            if j >= 1:
                g, t0 = divmod((j - 1) * 2, NT_)
                pv(g, t0)
                if pat == 5:
                    for d in sched.get(j, []): d()
                pv(g, t0 + 1)
            elif pat == 5:
                for d in sched.get(j, []): d()
            if pat == 4:
                for d in sched.get(j, []): d()
        sq_ref[...] = sq_next
        for d in tail:
            d()
        oproj(3)

    @pl.when(jnp.logical_not(fast))
    def _():
        for d in ffn:
            d()
        kb = kvT_ref[0:DH, :].astype(bf16)

        def grp(g, _):
            qg = jnp.concatenate(
                [qT_ref[i, pl.ds(pl.multiple_of((g * GH + u) * DH, DH), DH), :] for u in range(GH)], axis=1).astype(bf16)
            s = lax.dot_general(kb, qg, TN, preferred_element_type=f32)
            m = jnp.max(s, axis=0, keepdims=True)
            p = jnp.exp2(s - m)
            l = jnp.sum(p, axis=0, keepdims=True)
            o = jnp.dot(vT_ref[...], p.astype(bf16), preferred_element_type=f32)
            res = o * (1.0 / l)
            for u in range(GH):
                hr = pl.multiple_of((g * GH + u) * DH, DH)
                oT_ref[pl.ds(hr, DH), :] = res[:, u * TQ:(u + 1) * TQ] * cv_ref[...]
            return 0
        lax.fori_loop(0, NG, grp, 0)
        for n in range(4):
            oproj(n)


@jax.jit
def pallas_parallel_sum__grouped_kv_mqa__dense_activation_silu__prompt_kernel(A_x, A_wq, A_wk, A_wv, A_wo, B_x, B_w1, B_w2):
    if True:
        pat, ntail, LC, wstart = 3, 2, 256, 2
        nsteps = A_x.shape[1] // TQ
        B, S, D = A_x.shape
        F = B_w1.shape[1]
        x = A_x.reshape(S, D)
        full = lambda shp: pl.BlockSpec(shp, lambda i: (0,) * len(shp))
        hbm = pl.BlockSpec(memory_space=pl.ANY)
        out = pl.pallas_call(
            functools.partial(_kernel, S=S, D=D, F=F, pat=pat, ntail=ntail, LC=LC, wstart=wstart),
            grid=(nsteps,),
            in_specs=[hbm, hbm, full((DH, D)), full((DH, D)), hbm, hbm, hbm],
            out_specs=pl.BlockSpec((TQ, D), lambda i: (i, 0)),
            out_shape=jax.ShapeDtypeStruct((S, D), A_x.dtype),
            scratch_shapes=[
                pltpu.VMEM((S, D), bf16),
                pltpu.VMEM((D, D), bf16),
                pltpu.VMEM((D, D), bf16),
                pltpu.VMEM((D, F), bf16),
                pltpu.VMEM((F, D), bf16),
                pltpu.SemaphoreType.DMA((S // LC + 4,)),
                pltpu.VMEM((S, D), bf16),
                pltpu.VMEM((D + 2 * DH, D), bf16),
                pltpu.VMEM((2 * DH, S), f32),
                pltpu.VMEM((S, 128), jnp.int8),
                pltpu.VMEM((DH, S), bf16),
                pltpu.VMEM((DH, 128), f32),
                pltpu.VMEM((DH, 128), f32),
                pltpu.VMEM((S // TQ, D, TQ), f32),
                pltpu.VMEM((NG, 64, W), jnp.int8),
                pltpu.VMEM((8, TQ), f32),
                pltpu.VMEM((DH, TQ), f32),
                pltpu.VMEM((D, TQ), f32),
                pltpu.VMEM((TQ, F), bf16),
                pltpu.VMEM((TQ, D), f32),
                pltpu.SMEM((1,), jnp.int32),
            ],
            compiler_params=pltpu.CompilerParams(dimension_semantics=("arbitrary",), vmem_limit_bytes=100 * 1024 * 1024),
        )(x, A_wq, A_wk.T, A_wv.T, A_wo, B_w1, B_w2)
        return out.reshape(B, S, D)
```

```python
import functools
import jax, jax.numpy as jnp
from jax import lax
from jax.experimental import pallas as pl
from jax.experimental.pallas import tpu as pltpu

H = 32
DH = 16
LOG2E = 1.4426950408889634
TQ = 128
HW = 2 * TQ
NP = H // 2
KD = 96
ALPHA = 16.0
BETA = 16.0
BOUND = 48.0
f32 = jnp.float32
bf16 = jnp.bfloat16
NT = (((1,), (1,)), ((), ()))
TN = (((0,), (0,)), ((), ()))
P_ = functools.partial


def _rint(x):
    return jnp.round(x).astype(jnp.int32)


def _rev16(a, t):
    return jnp.concatenate([a[t * 128 + (7 - b) * 16: t * 128 + (8 - b) * 16] for b in range(8)], axis=0)


def _kernel(x_hbm, wq_hbm, wkT_ref, wvT_ref, wo_hbm, w1_hbm, w2_hbm, o_ref,
            x_ref, wq_ref, wo_ref, w1_ref, w2_ref, sems,
            xn_ref, wT_ref, kvT_ref, k8_ref, vT_ref, cv_ref, qT_ref, q8_ref, sq_ref, qs_ref, oT_ref, h_ref, acc_ref,
            pc_ref, sc_ref, lc_ref, flag_ref, *, S, D, F, LC, wstart, l1, oo, o3, f2lag):
    i = pl.program_id(0)
    nblk = S // TQ
    NCH = S // LC
    NKT = S // 128
    NF = F // 128

    def quant(blk, hp):
        q2 = qT_ref[blk, hp * 2 * DH:(hp + 1) * 2 * DH, :].reshape(2, DH, TQ) * qs_ref[blk][None]
        q2i = _rint(q2)
        q2f = q2i.astype(f32)
        qa = q2i >> 1
        qb = q2i - qa
        dq = _rint((q2 - q2f) * ALPHA)
        rq = _rint(q2f * (1.0 / BETA))
        main = jnp.concatenate([qa, qb], axis=1).astype(jnp.int8)
        corr = jnp.concatenate([dq, rq], axis=1).astype(jnp.int8)
        for u in range(2):
            q8_ref[hp, 0:32, u * TQ:(u + 1) * TQ] = main[u]
            q8_ref[hp, 32:64, u * TQ:(u + 1) * TQ] = corr[u]

    @pl.when(i == 0)
    def _():
        xcp = [pltpu.make_async_copy(x_hbm.at[pl.ds(c * LC, LC)], x_ref.at[pl.ds(c * LC, LC)], sems.at[c])
               for c in range(NCH)]
        wqcp = pltpu.make_async_copy(wq_hbm, wq_ref, sems.at[NCH])
        wcp = [pltpu.make_async_copy(s_, d_, sems.at[NCH + 1 + n])
               for n, (s_, d_) in enumerate(((w1_hbm, w1_ref), (w2_hbm, w2_ref), (wo_hbm, wo_ref)))]
        xcp[0].start()
        wqcp.start()
        for c in range(1, NCH):
            xcp[c].start()
        pc_ref[...] = jnp.zeros_like(pc_ref)
        sc_ref[...] = jnp.zeros_like(sc_ref)
        lc_ref[...] = jnp.ones_like(lc_ref)
        acc_ref[...] = jnp.zeros_like(acc_ref)
        oT_ref[...] = jnp.zeros_like(oT_ref)

        def ln(c):
            x = x_ref[c * LC:(c + 1) * LC, :].astype(f32)
            m = jnp.mean(x, axis=-1, keepdims=True)
            xc = x - m
            v = jnp.mean(xc * xc, axis=-1, keepdims=True)
            xn_ref[c * LC:(c + 1) * LC, :] = (xc * lax.rsqrt(v + 1e-5)).astype(bf16)

        def proj(c, qn):
            y = lax.dot_general(wT_ref[...], xn_ref[c * LC:(c + 1) * LC, :], NT, preferred_element_type=f32)
            kvT_ref[:, c * LC:(c + 1) * LC] = y[D:D + 2 * DH]
            for t in range(LC // TQ):
                blk = c * (LC // TQ) + t
                qT = y[0:D, t * TQ:(t + 1) * TQ] * (DH ** -0.5 * LOG2E)
                qT_ref[blk] = qT
                q3 = qT.reshape(H, DH, TQ)
                qs_ref[blk] = jnp.max(jnp.abs(q3), axis=0)
                q2 = jnp.sum(q3 * q3, axis=1)
                qn = q2 if qn is None else jnp.maximum(qn, q2)
            return qn

        xcp[0].wait()
        ln(0)
        wqcp.wait()
        wT_ref[0:D, :] = wq_ref[...].T
        wT_ref[D:D + DH, :] = wkT_ref[...]
        wT_ref[D + DH:D + 2 * DH, :] = wvT_ref[...]
        qn = None
        for c in range(NCH):
            if c == wstart:
                for cp in wcp:
                    cp.start()
            if c + 1 < NCH:
                xcp[c + 1].wait()
            qn = proj(c, qn)
            if c + 1 < NCH:
                ln(c + 1)

        kvT = kvT_ref[...]
        cmax = jnp.max(jnp.abs(kvT), axis=1, keepdims=True)
        cmax = jnp.where(cmax > 0, cmax, 1.0)
        cb = jnp.broadcast_to(cmax, (2 * DH, 128))
        ck = cb[0:DH]
        cv_ref[...] = cb[DH:2 * DH]
        kvn = kvT * (1.0 / cmax)
        vT_ref[...] = kvn[DH:2 * DH].astype(bf16)
        kT = kvT[0:DH]
        kn2 = jnp.sum(kT * kT, axis=0, keepdims=True)
        flag_ref[0] = (jnp.max(qn) * jnp.max(kn2) <= BOUND * BOUND).astype(jnp.int32)
        k2 = kvn[0:DH] * 254.0
        k2i = _rint(k2)
        ka = k2i >> 1
        kb = k2i - ka
        dk = _rint((k2 - k2i.astype(f32)) * BETA)
        rk = _rint(k2 * (1.0 / ALPHA))
        ka, kb, dk, rk = [a.astype(f32).astype(bf16) for a in (ka, kb, dk, rk)]
        zz = jnp.zeros_like(ka)
        aT = jnp.concatenate([ka, kb, kb, ka, rk, dk, zz, zz], axis=0)
        r = lax.broadcasted_iota(jnp.int32, (128, 128), 0)
        c_ = lax.broadcasted_iota(jnp.int32, (128, 128), 1)
        perm = jnp.where(c_ == (7 - r // 16) * 16 + r % 16, 1.0, 0.0).astype(bf16)
        for t in range(NKT):
            kt = lax.dot_general(perm, aT[:, t * 128:(t + 1) * 128], NT, preferred_element_type=f32)
            k8_ref[t * 128:(t + 1) * 128, :] = kt.astype(jnp.int32).astype(jnp.int8)
        am = jnp.max(qs_ref[...] * ck[None], axis=1, keepdims=True)
        am = jnp.where(am > 0, am, 1.0)
        qs_ref[...] = ck[None] * (254.0 / am)
        sq_ref[...] = jnp.broadcast_to(am * (1.0 / (254.0 * 254.0)), (nblk, 8, TQ))
        for hp in range(NP):
            quant(0, hp)
        for cp in wcp:
            cp.wait()

    fast = flag_ref[0] > 0
    ib = jnp.minimum(i, nblk - 1)
    r0 = pl.multiple_of(ib * TQ, TQ)
    hold = {}

    def f1(c, half):
        y = jnp.dot(xn_ref[pl.ds(r0, TQ), half * 256:(half + 1) * 256],
                    w1_ref[half * 256:(half + 1) * 256, c * 128:(c + 1) * 128], preferred_element_type=f32)
        if half == 0:
            hold[c] = y
        else:
            u = 0.5 * (y + hold.pop(c))
            h_ref[:, c * 128:(c + 1) * 128] = (u + u * jnp.tanh(u)).astype(bf16)

    def f2(c, half):
        cs = slice(half * 256, (half + 1) * 256)
        y = jnp.dot(h_ref[:, c * 128:(c + 1) * 128], w2_ref[c * 128:(c + 1) * 128, cs], preferred_element_type=f32)
        if c == 0:
            acc_ref[:, cs] = y + x_ref[pl.ds(r0, TQ), cs].astype(f32)
        else:
            acc_ref[:, cs] += y

    def op(n, half):
        cs = slice(half * 256, (half + 1) * 256)
        if half == 0:
            hold[("o", n)] = oT_ref[n * 128:(n + 1) * 128, :].T.astype(bf16)
            o = hold[("o", n)]
        else:
            o = hold.pop(("o", n))
        y = jnp.dot(o, wo_ref[n * 128:(n + 1) * 128, cs], preferred_element_type=f32)
        if n == 3:
            o_ref[:, cs] = (acc_ref[:, cs] + y).astype(o_ref.dtype)
        else:
            acc_ref[:, cs] += y

    def finish(hp, o, l):
        res = o * (1.0 / jnp.sum(l, axis=0, keepdims=True))
        for u in range(2):
            h = hp * 2 + u
            oT_ref[h * DH:(h + 1) * DH, :] = res[:, u * TQ:(u + 1) * TQ] * cv_ref[...]

    units = []
    for g in range(NP // 2):
        for tq_ in range(NKT // 4):
            for half in range(2):
                units.append((2 * g + half, tq_ * 4))
    nu = len(units)
    carry_a = [(NP - 2, NKT - 1)]
    carry_b = [(NP - 1, NKT - 5 + t) for t in range(5)]
    carry = carry_a + carry_b

    class Att:
        def __init__(self):
            self.pt, self.st, self.ls, self.cnt = {}, {}, {}, {}

        def load_carry(self):
            for n, hp in enumerate((NP - 2, NP - 1)):
                self.st[("c", hp)] = sc_ref[n]
                self.ls[("c", hp)] = lc_ref[n]
                self.cnt[("c", hp)] = NKT - sum(1 for c in carry if c[0] == hp)

        def pv(self, key, t):
            if isinstance(key, tuple):
                p = pc_ref[carry.index((key[1], t))]
                hp = key[1]
            else:
                p = self.pt.pop((key, t))
                hp = key
            o = jnp.dot(vT_ref[:, t * 128:(t + 1) * 128], p, preferred_element_type=f32)
            self.st[key] = o if key not in self.st else o + self.st[key]
            self.cnt[key] = self.cnt.get(key, 0) + 1
            if self.cnt[key] == NKT:
                finish(hp, self.st.pop(key), self.ls.pop(key))

    @pl.when(jnp.logical_and(fast, i < nblk))
    def _():
        A = Att()
        A.load_carry()
        nxt = jnp.minimum(i + 1, nblk - 1)
        sq = jnp.concatenate([sq_ref[ib]] * 2, axis=1)

        def qk(hp, t0):
            q8 = q8_ref[hp]
            wgt = jnp.concatenate([q8[0:32], q8[0:32], q8[32:64]], axis=0)
            s = jnp.dot(k8_ref[t0 * 128:(t0 + 4) * 128, 0:KD], wgt, preferred_element_type=jnp.int32)
            s = s.astype(f32).reshape(64, 8, HW) * sq[None]
            p = jnp.exp2(s)
            l = jnp.sum(p, axis=0)
            A.ls[hp] = l if t0 == 0 else A.ls[hp] + l
            p = p.reshape(512, HW)
            for t in range(4):
                A.pt[(hp, t0 + t)] = _rev16(p, t).astype(bf16)

        dense = []
        for c in range(NF + f2lag):
            if c < NF:
                dense += [P_(f1, c, 0), P_(f1, c, 1)]
            if c >= f2lag:
                dense += [P_(f2, c - f2lag, 0), P_(f2, c - f2lag, 1)]
        opq = [(o3 + half, P_(op, 3, half)) for half in range(2)]
        opq += [(oo + 16 * n + half, P_(op, n, half)) for n in range(3) for half in range(2)]
        slot = []
        for j in range(nu):
            slot.append(opq.pop(0)[1] if opq and j >= opq[0][0] else dense.pop(0))
        assert not dense and not opq
        assert 2 * f2lag >= o3

        cQ, cP, cD = 256, 32, 128
        seqs = [[], []]
        tl = [[(("c", hp), t) for hp, t in carry_a], [(("c", hp), t) for hp, t in carry_b]]

        def phase(a):
            for ch in "PPDPP":
                if ch == "D":
                    seqs[a].append((cD, "D", slot.pop(0)))
                else:
                    seqs[a].append((cP, "P", tl[a].pop(0)))
        phase(1)
        for j in range(nu):
            hp, t0 = units[j]
            a = j % 2
            seqs[a].append((cQ, "Q", j))
            tl[a] += [(hp, t0 + t) for t in range(4)]
            if j < nu - 1:
                phase(a)
        assert tl[0] == carry_a and tl[1] == carry_b
        load = [0, l1]
        idx = [0, 0]
        while idx[0] < len(seqs[0]) or idx[1] < len(seqs[1]):
            a = 0 if idx[1] >= len(seqs[1]) or (idx[0] < len(seqs[0]) and load[0] <= load[1]) else 1
            c, kind, pay = seqs[a][idx[a]]
            idx[a] += 1
            load[a] += c
            if kind == "Q":
                qk(*units[pay])
                if units[pay][1] == NKT - 4:
                    quant(nxt, units[pay][0])
            elif kind == "P":
                A.pv(*pay)
            else:
                pay()
        for n, key in enumerate(carry):
            pc_ref[n] = A.pt.pop(key)
        for n, hp in enumerate((NP - 2, NP - 1)):
            sc_ref[n] = A.st.pop(hp)
            lc_ref[n] = A.ls.pop(hp)

    @pl.when(jnp.logical_and(fast, i == nblk))
    def _():
        A = Att()
        A.load_carry()
        for hp, t in carry:
            A.pv(("c", hp), t)
        op(3, 0)
        op(3, 1)

    @pl.when(jnp.logical_not(fast))
    def _():
        op(3, 0)
        op(3, 1)

        @pl.when(i < nblk)
        def _():
            for c in range(NF):
                f1(c, 0)
                f1(c, 1)
                f2(c, 0)
                f2(c, 1)
            kb = kvT_ref[0:DH, :].astype(bf16)

            def pair(hp, _):
                qg = jnp.concatenate(
                    [qT_ref[ib, pl.ds(pl.multiple_of((hp * 2 + u) * DH, DH), DH), :] for u in range(2)],
                    axis=1).astype(bf16)
                s = lax.dot_general(kb, qg, TN, preferred_element_type=f32)
                m = jnp.max(s, axis=0, keepdims=True)
                p = jnp.exp2(s - m)
                l = jnp.sum(p, axis=0, keepdims=True)
                o = jnp.dot(vT_ref[...], p.astype(bf16), preferred_element_type=f32)
                res = o * (1.0 / l)
                for u in range(2):
                    hr = pl.multiple_of((hp * 2 + u) * DH, DH)
                    oT_ref[pl.ds(hr, DH), :] = res[:, u * TQ:(u + 1) * TQ] * cv_ref[...]
                return 0
            lax.fori_loop(0, NP, pair, 0)
            for n in range(3):
                op(n, 0)
                op(n, 1)


@jax.jit
def pallas_parallel_sum__grouped_kv_mqa__dense_activation_silu__prompt_kernel(A_x, A_wq, A_wk, A_wv, A_wo, B_x, B_w1, B_w2):
    LC = 256
    wstart = 2
    l1 = 0
    oo = 20
    o3 = 4
    f2lag = 2
    B, S, D = A_x.shape
    F = B_w1.shape[1]
    nblk = S // TQ
    x = A_x.reshape(S, D)
    full = lambda shp: pl.BlockSpec(shp, lambda i: (0,) * len(shp))
    hbm = pl.BlockSpec(memory_space=pl.ANY)
    out = pl.pallas_call(
        functools.partial(_kernel, S=S, D=D, F=F, LC=LC, wstart=wstart, l1=l1, oo=oo, o3=o3, f2lag=f2lag),
        grid=(nblk + 1,),
        in_specs=[hbm, hbm, full((DH, D)), full((DH, D)), hbm, hbm, hbm],
        out_specs=pl.BlockSpec((TQ, D), lambda i: (jnp.maximum(i - 1, 0), 0)),
        out_shape=jax.ShapeDtypeStruct((S, D), A_x.dtype),
        scratch_shapes=[
            pltpu.VMEM((S, D), bf16),
            pltpu.VMEM((D, D), bf16),
            pltpu.VMEM((D, D), bf16),
            pltpu.VMEM((D, F), bf16),
            pltpu.VMEM((F, D), bf16),
            pltpu.SemaphoreType.DMA((S // LC + 4,)),
            pltpu.VMEM((S, D), bf16),
            pltpu.VMEM((D + 2 * DH, D), bf16),
            pltpu.VMEM((2 * DH, S), f32),
            pltpu.VMEM((S, 128), jnp.int8),
            pltpu.VMEM((DH, S), bf16),
            pltpu.VMEM((DH, 128), f32),
            pltpu.VMEM((nblk, D, TQ), f32),
            pltpu.VMEM((NP, 64, HW), jnp.int8),
            pltpu.VMEM((nblk, 8, TQ), f32),
            pltpu.VMEM((nblk, DH, TQ), f32),
            pltpu.VMEM((D, TQ), f32),
            pltpu.VMEM((TQ, F), bf16),
            pltpu.VMEM((TQ, D), f32),
            pltpu.VMEM((6, 128, HW), bf16),
            pltpu.VMEM((2, DH, HW), f32),
            pltpu.VMEM((2, 8, HW), f32),
            pltpu.SMEM((1,), jnp.int32),
        ],
        compiler_params=pltpu.CompilerParams(dimension_semantics=("arbitrary",), vmem_limit_bytes=100 * 1024 * 1024),
    )(x, A_wq, A_wk.T, A_wv.T, A_wo, B_w1, B_w2)
    return out.reshape(B, S, D)
```

```python
import functools

import jax
import jax.numpy as jnp
from jax import lax
import jax.experimental.pallas as pl
import jax.experimental.pallas.tpu as pltpu

H = 32
DH = 16
TQ = 128
NB = 2
HW = 2 * TQ
NP = H // 2
KD = 6 * DH
LC = 256
QMAX = 254.0
ALPHA = 16.0
BOUND = 48.0
LOG2E = 1.4426950408889634

f32 = jnp.float32
bf16 = jnp.bfloat16
NT = (((1,), (1,)), ((), ()))
TN = (((0,), (0,)), ((), ()))
P_ = functools.partial


def _rint(x):
    return jnp.round(x).astype(jnp.int32)


def _limbs(v):
    vi = _rint(v)
    vf = vi.astype(f32)
    a = vi >> 1
    return a, vi - a, vf, _rint((v - vf) * ALPHA)


def _rev16(a, t):
    return jnp.concatenate(
        [a[t * 128 + (7 - b) * 16: t * 128 + (8 - b) * 16] for b in range(8)], axis=0)


def _kernel(x_hbm, wq_hbm, wkT_ref, wvT_ref, wo_hbm, w1_hbm, w2_hbm, o_ref,
            x_ref, wq_ref, wo_ref, w1_ref, w2_ref, sems,
            xn_ref, wT_ref, kvT_ref, k8_ref, vT_ref, cv_ref, qT_ref, q8_ref, sq_ref, qs_ref,
            oT_ref, h_ref, acc_ref, pc_ref, sc_ref, lc_ref, stg_ref, flag_ref, *, S, D, F):
    i = pl.program_id(0)
    nblk = S // TQ
    nst = nblk // NB
    NCH = S // LC
    NKT = S // 128
    NF = F // 128
    HD = D // 2

    def quant(blk, hp):
        q2 = qT_ref[blk, hp * 2 * DH:(hp + 1) * 2 * DH, :].reshape(2, DH, TQ) * qs_ref[blk][None]
        qa, qb, qf, dq = _limbs(q2)
        rq = _rint(qf * (1.0 / ALPHA))
        main = jnp.concatenate([qa, qb], axis=1).astype(jnp.int8)
        corr = jnp.concatenate([dq, rq], axis=1).astype(jnp.int8)
        for u in range(2):
            q8_ref[hp, 0:32, u * TQ:(u + 1) * TQ] = main[u]
            q8_ref[hp, 32:64, u * TQ:(u + 1) * TQ] = corr[u]

    @pl.when(i == 0)
    def _():
        xcp = [pltpu.make_async_copy(x_hbm.at[pl.ds(c * LC, LC)], x_ref.at[pl.ds(c * LC, LC)],
                                     sems.at[c]) for c in range(NCH)]
        wqcp = pltpu.make_async_copy(wq_hbm, wq_ref, sems.at[NCH])
        wcp = [pltpu.make_async_copy(s_, d_, sems.at[NCH + 1 + n])
               for n, (s_, d_) in enumerate(((w1_hbm, w1_ref), (w2_hbm, w2_ref), (wo_hbm, wo_ref)))]
        xcp[0].start()
        wqcp.start()
        for c in range(1, NCH):
            xcp[c].start()
        pc_ref[...] = jnp.zeros_like(pc_ref)
        sc_ref[...] = jnp.zeros_like(sc_ref)
        lc_ref[...] = jnp.ones_like(lc_ref)
        acc_ref[...] = jnp.zeros_like(acc_ref)
        oT_ref[...] = jnp.zeros_like(oT_ref)
        stg_ref[...] = jnp.zeros_like(stg_ref)

        def ln(c):
            x = x_ref[c * LC:(c + 1) * LC, :].astype(f32)
            m = jnp.mean(x, axis=-1, keepdims=True)
            xc = x - m
            v = jnp.mean(xc * xc, axis=-1, keepdims=True)
            xn_ref[c * LC:(c + 1) * LC, :] = (xc * lax.rsqrt(v + 1e-5)).astype(bf16)

        def proj(c, qn):
            y = lax.dot_general(wT_ref[...], xn_ref[c * LC:(c + 1) * LC, :], NT,
                                preferred_element_type=f32)
            kvT_ref[:, c * LC:(c + 1) * LC] = y[D:D + 2 * DH]
            for t in range(LC // TQ):
                blk = c * (LC // TQ) + t
                qT = y[0:D, t * TQ:(t + 1) * TQ] * (DH ** -0.5 * LOG2E)
                qT_ref[blk] = qT
                q3 = qT.reshape(H, DH, TQ)
                qs_ref[blk] = jnp.max(jnp.abs(q3), axis=0)
                q2 = jnp.sum(q3 * q3, axis=1)
                qn = q2 if qn is None else jnp.maximum(qn, q2)
            return qn

        xcp[0].wait()
        ln(0)
        wqcp.wait()
        wT_ref[0:D, :] = wq_ref[...].T
        wT_ref[D:D + DH, :] = wkT_ref[...]
        wT_ref[D + DH:D + 2 * DH, :] = wvT_ref[...]
        qn = None
        waited = 1
        for c in range(NCH):
            if c == 1:
                for cp in wcp:
                    cp.start()
            if waited <= c + 1 < NCH:
                upto = min(2 * waited, NCH)
                for cc in range(waited, upto):
                    xcp[cc].wait()
                waited = upto
            qn = proj(c, qn)
            if c + 1 < NCH:
                ln(c + 1)

        kvT = kvT_ref[...]
        cmax = jnp.max(jnp.abs(kvT), axis=1, keepdims=True)
        kvn = kvT * jnp.where(cmax > 0, 1.0 / jnp.where(cmax > 0, cmax, 1.0), 0.0)
        cb = jnp.broadcast_to(cmax, (2 * DH, 128))
        ck = cb[0:DH]
        cv_ref[...] = cb[DH:2 * DH]
        vT_ref[...] = kvn[DH:2 * DH].astype(bf16)
        kT = kvT[0:DH]
        kn = jnp.sum(kT * kT, axis=0, keepdims=True)
        flag_ref[0] = (jnp.max(qn) * jnp.max(kn) <= BOUND * BOUND).astype(jnp.int32)
        k2 = kvn[0:DH] * QMAX
        ka, kb, _, dk = _limbs(k2)
        rk = _rint(k2 * (1.0 / ALPHA))
        ka, kb, dk, rk = [a.astype(f32).astype(bf16) for a in (ka, kb, dk, rk)]
        zz = jnp.zeros_like(ka)
        aT = jnp.concatenate([ka, kb, kb, ka, rk, dk, zz, zz], axis=0)
        r = lax.broadcasted_iota(jnp.int32, (128, 128), 0)
        c_ = lax.broadcasted_iota(jnp.int32, (128, 128), 1)
        perm = jnp.where(c_ == (7 - r // 16) * 16 + r % 16, 1.0, 0.0).astype(bf16)
        for t in range(NKT):
            kt = lax.dot_general(perm, aT[:, t * 128:(t + 1) * 128], NT, preferred_element_type=f32)
            k8_ref[t * 128:(t + 1) * 128, :] = kt.astype(jnp.int32).astype(jnp.int8)
        am = jnp.max(qs_ref[...] * ck[None], axis=1, keepdims=True)
        am = jnp.maximum(am, 2.0 ** -20)
        qs_ref[...] = ck[None] * (QMAX / am)
        sq_ref[...] = jnp.broadcast_to(am * (1.0 / (QMAX * QMAX)), (nblk, 8, TQ))
        for hp in range(NP):
            quant(0, hp)
        for cp in wcp:
            cp.wait()

    fast = flag_ref[0] > 0
    ist = jnp.minimum(i, nst - 1)
    hold = {}

    def rows(b):
        return pl.ds(pl.multiple_of((ist * NB + b) * TQ, TQ), TQ)

    def silu(y):
        u = 0.5 * y
        return u + u * jnp.tanh(u)

    def f1(b, c, half):
        ks = slice(half * HD, (half + 1) * HD)
        y = jnp.dot(xn_ref[rows(b), ks], w1_ref[ks, c * 128:(c + 1) * 128],
                    preferred_element_type=f32)
        if half == 0:
            hold[c] = y
        else:
            h_ref[:, c * 128:(c + 1) * 128] = silu(y + hold.pop(c)).astype(bf16)

    def f2(b, c, half):
        cs = slice(half * HD, (half + 1) * HD)
        y = jnp.dot(h_ref[:, c * 128:(c + 1) * 128], w2_ref[c * 128:(c + 1) * 128, cs],
                    preferred_element_type=f32)
        if c == 0:
            acc_ref[:, cs] = y + x_ref[rows(b), cs].astype(f32)
        else:
            acc_ref[:, cs] += y

    def op(b, n, half):
        cs = slice(half * HD, (half + 1) * HD)
        if half == 0:
            hold[("o", n)] = oT_ref[n * 128:(n + 1) * 128, :].T.astype(bf16)
            o = hold[("o", n)]
        else:
            o = hold.pop(("o", n))
        y = jnp.dot(o, wo_ref[n * 128:(n + 1) * 128, cs], preferred_element_type=f32)
        if n < 3:
            acc_ref[:, cs] += y
        else:
            res = (acc_ref[:, cs] + y).astype(o_ref.dtype)
            if b < NB - 1:
                stg_ref[b * TQ:(b + 1) * TQ, cs] = res
            else:
                o_ref[b * TQ:(b + 1) * TQ, cs] = res
                o_ref[0:b * TQ, cs] = stg_ref[0:b * TQ, cs]

    units = [(2 * g + half, 4 * t4)
             for g in range(NP // 2) for t4 in range(NKT // 4) for half in range(2)]
    nu = len(units)
    carry_a = [(NP - 2, NKT - 1)]
    carry_b = [(NP - 1, NKT - 4 + t) for t in range(4)]
    carry = carry_a + carry_b

    class Att:
        def __init__(self):
            self.pt, self.st, self.ls, self.cnt = {}, {}, {}, {}
            for n, hp in enumerate((NP - 2, NP - 1)):
                self.st[("c", hp)] = sc_ref[n]
                self.ls[("c", hp)] = lc_ref[n]
                self.cnt[("c", hp)] = NKT - sum(1 for c in carry if c[0] == hp)

        def pv(self, key, t):
            if isinstance(key, tuple):
                hp = key[1]
                p = pc_ref[carry.index((hp, t))]
            else:
                hp = key % NP
                p = self.pt.pop((key, t))
            o = jnp.dot(vT_ref[:, t * 128:(t + 1) * 128], p, preferred_element_type=f32)
            self.st[key] = o if key not in self.st else o + self.st[key]
            self.cnt[key] = self.cnt.get(key, 0) + 1
            if self.cnt[key] == NKT:
                l = jnp.sum(self.ls.pop(key), axis=0, keepdims=True)
                res = self.st.pop(key) * (1.0 / l)
                for u in range(2):
                    h = hp * 2 + u
                    oT_ref[h * DH:(h + 1) * DH, :] = res[:, u * TQ:(u + 1) * TQ] * cv_ref[...]

    @pl.when(jnp.logical_and(fast, i < nst))
    def _():
        A = Att()
        sqs = {}

        def qk(b, hp, t0):
            if b not in sqs:
                sqs[b] = jnp.concatenate([sq_ref[ist * NB + b]] * 2, axis=1)
            q8 = q8_ref[hp]
            wgt = jnp.concatenate([q8[0:32], q8[0:32], q8[32:64]], axis=0)
            s = jnp.dot(k8_ref[t0 * 128:(t0 + 4) * 128, 0:KD], wgt,
                        preferred_element_type=jnp.int32)
            p = jnp.exp2(s.astype(f32).reshape(64, 8, HW) * sqs[b][None])
            l = jnp.sum(p, axis=0)
            key = b * NP + hp
            A.ls[key] = l if t0 == 0 else A.ls[key] + l
            p = p.reshape(512, HW)
            for t in range(4):
                A.pt[(key, t0 + t)] = _rev16(p, t).astype(bf16)

        slot = []
        for b in range(NB):
            dense = []
            for c in range(NF + 2):
                if c < NF:
                    dense += [P_(f1, b, c, 0), P_(f1, b, c, 1)]
                if c >= 2:
                    dense += [P_(f2, b, c - 2, 0), P_(f2, b, c - 2, 1)]
            opq = [(3 + half, P_(op, (b - 1) % NB, 3, half)) for half in range(2)]
            opq += [(22 + 16 * n + half, P_(op, b, n, half)) for n in range(3) for half in range(2)]
            for j in range(nu):
                slot.append(opq.pop(0)[1] if opq and j >= opq[0][0] else dense.pop(0))
            assert not dense and not opq

        cQ, cP, cD = 256, 32, 128
        seqs = [[], []]
        tl = [[(("c", hp), t) for hp, t in carry_a], [(("c", hp), t) for hp, t in carry_b]]

        def phase(a, pat):
            for ch in pat:
                if ch == "D":
                    seqs[a].append((cD, "D", slot.pop(0)))
                else:
                    seqs[a].append((cP, "P", tl[a].pop(0)))

        phase(1, "PDPP")
        for jj in range(NB * nu):
            b, j = divmod(jj, nu)
            hp, t0 = units[j]
            seqs[j % 2].append((cQ, "Q", (b, hp, t0)))
            tl[j % 2] += [(b * NP + hp, t0 + t) for t in range(4)]
            phase(j % 2, "PPDPP" if jj < NB * nu - 1 else "P")
        busy = [0, 0]
        idx = [0, 0]
        while idx[0] < len(seqs[0]) or idx[1] < len(seqs[1]):
            first = idx[1] >= len(seqs[1]) or (idx[0] < len(seqs[0]) and busy[0] <= busy[1])
            a = 0 if first else 1
            cost, kind, pay = seqs[a][idx[a]]
            idx[a] += 1
            busy[a] += cost
            if kind == "Q":
                qk(*pay)
                if pay[2] == NKT - 4:
                    quant(jnp.minimum(ist * NB + pay[0] + 1, nblk - 1), pay[1])
            elif kind == "P":
                A.pv(*pay)
            else:
                pay()
        off = (NB - 1) * NP
        for n, (hp, t) in enumerate(carry):
            pc_ref[n] = A.pt.pop((off + hp, t))
        for n, hp in enumerate((NP - 2, NP - 1)):
            sc_ref[n] = A.st.pop(off + hp)
            lc_ref[n] = A.ls.pop(off + hp)

    @pl.when(jnp.logical_and(fast, i == nst))
    def _():
        A = Att()
        for hp, t in carry:
            A.pv(("c", hp), t)
        op(NB - 1, 3, 0)
        op(NB - 1, 3, 1)

    @pl.when(jnp.logical_not(fast))
    def _():
        o_ref[...] = stg_ref[...]

        @pl.when(i < nst)
        def _():
            kb = kvT_ref[0:DH, :].astype(bf16)

            def sub(b, carry_):
                def pair(hp, carry__):
                    qg = jnp.concatenate(
                        [qT_ref[ist * NB + b, pl.ds(pl.multiple_of((hp * 2 + u) * DH, DH), DH), :]
                         for u in range(2)], axis=1).astype(bf16)
                    s = lax.dot_general(kb, qg, TN, preferred_element_type=f32)
                    p = jnp.exp2(s - jnp.max(s, axis=0, keepdims=True))
                    l = jnp.sum(p, axis=0, keepdims=True)
                    o = jnp.dot(vT_ref[...], p.astype(bf16), preferred_element_type=f32)
                    res = o * (1.0 / l)
                    for u in range(2):
                        hr = pl.multiple_of((hp * 2 + u) * DH, DH)
                        oT_ref[pl.ds(hr, DH), :] = res[:, u * TQ:(u + 1) * TQ] * cv_ref[...]
                    return carry__
                lax.fori_loop(0, NP, pair, 0)
                hh = silu(jnp.dot(xn_ref[rows(b), :], w1_ref[...], preferred_element_type=f32))
                y = jnp.dot(hh.astype(bf16), w2_ref[...], preferred_element_type=f32)
                y = y + jnp.dot(oT_ref[...].T.astype(bf16), wo_ref[...], preferred_element_type=f32)
                y = y + x_ref[rows(b), :].astype(f32)
                stg_ref[pl.ds(pl.multiple_of(b * TQ, TQ), TQ), :] = y.astype(stg_ref.dtype)
                return carry_
            lax.fori_loop(0, NB, sub, 0)


@jax.jit
def pallas_parallel_sum__grouped_kv_mqa__dense_activation_silu__prompt_kernel(
    A_x: jax.Array,
    A_wq: jax.Array,
    A_wk: jax.Array,
    A_wv: jax.Array,
    A_wo: jax.Array,
    B_x: jax.Array,
    B_w1: jax.Array,
    B_w2: jax.Array,
):
    del B_x
    B, S, D = A_x.shape
    F = B_w1.shape[1]
    assert B == 1 and D == H * DH == 512 and S % (NB * TQ) == 0 and S % 512 == 0
    assert F % 128 == 0 and 4 * (F // 128) + 8 == NP * (S // 512)
    nblk = S // TQ
    small = pl.BlockSpec((DH, D), lambda i: (0, 0))
    hbm = pl.BlockSpec(memory_space=pl.ANY)
    out = pl.pallas_call(
        functools.partial(_kernel, S=S, D=D, F=F),
        grid=(nblk // NB + 1,),
        in_specs=[hbm, hbm, small, small, hbm, hbm, hbm],
        out_specs=pl.BlockSpec((NB * TQ, D), lambda i: (jnp.maximum(i - 1, 0), 0)),
        out_shape=jax.ShapeDtypeStruct((S, D), A_x.dtype),
        scratch_shapes=[
            pltpu.VMEM((S, D), bf16),
            pltpu.VMEM((D, D), bf16),
            pltpu.VMEM((D, D), bf16),
            pltpu.VMEM((D, F), bf16),
            pltpu.VMEM((F, D), bf16),
            pltpu.SemaphoreType.DMA((S // LC + 4,)),
            pltpu.VMEM((S, D), bf16),
            pltpu.VMEM((D + 2 * DH, D), bf16),
            pltpu.VMEM((2 * DH, S), f32),
            pltpu.VMEM((S, 128), jnp.int8),
            pltpu.VMEM((DH, S), bf16),
            pltpu.VMEM((DH, 128), f32),
            pltpu.VMEM((nblk, D, TQ), f32),
            pltpu.VMEM((NP, 64, HW), jnp.int8),
            pltpu.VMEM((nblk, 8, TQ), f32),
            pltpu.VMEM((nblk, DH, TQ), f32),
            pltpu.VMEM((D, TQ), f32),
            pltpu.VMEM((TQ, F), bf16),
            pltpu.VMEM((TQ, D), f32),
            pltpu.VMEM((5, 128, HW), bf16),
            pltpu.VMEM((2, DH, HW), f32),
            pltpu.VMEM((2, 8, HW), f32),
            pltpu.VMEM((NB * TQ, D), A_x.dtype),
            pltpu.SMEM((1,), jnp.int32),
        ],
        compiler_params=pltpu.CompilerParams(
            dimension_semantics=("arbitrary",), vmem_limit_bytes=64 * 1024 * 1024),
    )(A_x.reshape(S, D), A_wq, A_wk.T, A_wv.T, A_wo, B_w1, B_w2)
    return out.reshape(B, S, D)
```

```python
import functools

import jax
import jax.numpy as jnp
from jax import lax
import jax.experimental.pallas as pl
import jax.experimental.pallas.tpu as pltpu

H = 32
DH = 16
TQ = 128
NB = 2
HW = 2 * TQ
NP = H // 2
KD = 6 * DH
LC = 256
QMAX = 254.0
ALPHA = 16.0
BOUND = 48.0
LOG2E = 1.4426950408889634

f32 = jnp.float32
bf16 = jnp.bfloat16
NT = (((1,), (1,)), ((), ()))
TN = (((0,), (0,)), ((), ()))
P_ = functools.partial


def _rint(x):
    return jnp.round(x).astype(jnp.int32)


def _limbs(v):
    vi = _rint(v)
    vf = vi.astype(f32)
    a = vi >> 1
    return a, vi - a, vf, _rint((v - vf) * ALPHA)


def _rev16(a, t):
    return jnp.concatenate(
        [a[t * 128 + (7 - b) * 16: t * 128 + (8 - b) * 16] for b in range(8)], axis=0)


def _kernel(x_hbm, wq_hbm, wkT_hbm, wvT_hbm, wo_hbm, w1_hbm, w2_hbm, o_ref,
            x_ref, wq_ref, wo_ref, w1_ref, w2_ref, sems,
            xn_ref, wT_ref, kvT_ref, k8_ref, vT_ref, cv_ref, qT_ref, q8_ref, sq_ref, qs_ref,
            oT_ref, h_ref, acc_ref, pc_ref, sc_ref, lc_ref, stg_ref, flag_ref, *, S, D, F):
    i = pl.program_id(0)
    nblk = S // TQ
    nst = nblk // NB
    NCH = S // LC
    NKT = S // 128
    NF = F // 128
    HD = D // 2

    def quant(blk, hp):
        q2 = qT_ref[blk, hp * 2 * DH:(hp + 1) * 2 * DH, :].reshape(2, DH, TQ) * qs_ref[blk][None]
        qa, qb, qf, dq = _limbs(q2)
        rq = _rint(qf * (1.0 / ALPHA))
        main = jnp.concatenate([qa, qb], axis=1).astype(jnp.int8)
        corr = jnp.concatenate([dq, rq], axis=1).astype(jnp.int8)
        for u in range(2):
            q8_ref[hp, 0:32, u * TQ:(u + 1) * TQ] = main[u]
            q8_ref[hp, 32:64, u * TQ:(u + 1) * TQ] = corr[u]

    @pl.when(i == 0)
    def _():
        xcp = [pltpu.make_async_copy(x_hbm.at[pl.ds(c * LC, LC)], x_ref.at[pl.ds(c * LC, LC)],
                                     sems.at[c]) for c in range(NCH)]
        wqcp = pltpu.make_async_copy(wq_hbm, wq_ref, sems.at[NCH])
        wcp = [pltpu.make_async_copy(s_, d_, sems.at[NCH + 1 + n])
               for n, (s_, d_) in enumerate(((w1_hbm, w1_ref), (w2_hbm, w2_ref), (wo_hbm, wo_ref)))]
        kvcp = [pltpu.make_async_copy(s_, wT_ref.at[pl.ds(D + n * DH, DH)], sems.at[NCH + 4 + n])
                for n, s_ in enumerate((wkT_hbm, wvT_hbm))]
        xcp[0].start()
        wqcp.start()
        for cp in kvcp:
            cp.start()
        for c in range(1, NCH):
            xcp[c].start()
        pc_ref[...] = jnp.zeros_like(pc_ref)
        sc_ref[...] = jnp.zeros_like(sc_ref)
        lc_ref[...] = jnp.ones_like(lc_ref)
        acc_ref[...] = jnp.zeros_like(acc_ref)
        oT_ref[...] = jnp.zeros_like(oT_ref)
        stg_ref[...] = jnp.zeros_like(stg_ref)

        def ln(c):
            x = x_ref[c * LC:(c + 1) * LC, :].astype(f32)
            m = jnp.mean(x, axis=-1, keepdims=True)
            xc = x - m
            v = jnp.mean(xc * xc, axis=-1, keepdims=True)
            xn_ref[c * LC:(c + 1) * LC, :] = (xc * lax.rsqrt(v + 1e-5)).astype(bf16)

        def proj(c, qn):
            y = lax.dot_general(wT_ref[...], xn_ref[c * LC:(c + 1) * LC, :], NT,
                                preferred_element_type=f32)
            kvT_ref[:, c * LC:(c + 1) * LC] = y[D:D + 2 * DH]
            for t in range(LC // TQ):
                blk = c * (LC // TQ) + t
                qT = y[0:D, t * TQ:(t + 1) * TQ] * (DH ** -0.5 * LOG2E)
                qT_ref[blk] = qT
                q3 = qT.reshape(H, DH, TQ)
                qs_ref[blk] = jnp.max(jnp.abs(q3), axis=0)
                q2 = jnp.sum(q3 * q3, axis=1)
                qn = q2 if qn is None else jnp.maximum(qn, q2)
            return qn

        xcp[0].wait()
        ln(0)
        wqcp.wait()
        for cp in kvcp:
            cp.wait()
        wT_ref[0:D, :] = wq_ref[...].T
        qn = None
        waited = 1
        for c in range(NCH):
            if c == 1:
                for cp in wcp:
                    cp.start()
            if waited <= c + 1 < NCH:
                upto = min(2 * waited, NCH)
                for cc in range(waited, upto):
                    xcp[cc].wait()
                waited = upto
            qn = proj(c, qn)
            if c + 1 < NCH:
                ln(c + 1)

        kvT = kvT_ref[...]
        cmax = jnp.max(jnp.abs(kvT), axis=1, keepdims=True)
        cmax = jnp.maximum(cmax, 1e-30)
        kvn = kvT * (1.0 / cmax)
        cb = jnp.broadcast_to(cmax, (2 * DH, 128))
        ck = cb[0:DH]
        cv_ref[...] = cb[DH:2 * DH]
        vT_ref[...] = kvn[DH:2 * DH].astype(bf16)
        kT = kvT[0:DH]
        kn = jnp.sum(kT * kT, axis=0, keepdims=True)
        flag_ref[0] = (jnp.max(qn) * jnp.max(kn) <= BOUND * BOUND).astype(jnp.int32)
        k2 = kvn[0:DH] * QMAX
        ka, kb, _, dk = _limbs(k2)
        rk = _rint(k2 * (1.0 / ALPHA))
        ka, kb, dk, rk = [a.astype(f32).astype(bf16) for a in (ka, kb, dk, rk)]
        zz = jnp.zeros_like(ka)
        aT = jnp.concatenate([ka, kb, kb, ka, rk, dk, zz, zz], axis=0)
        r = lax.broadcasted_iota(jnp.int32, (128, 128), 0)
        c_ = lax.broadcasted_iota(jnp.int32, (128, 128), 1)
        perm = jnp.where(c_ == (7 - r // 16) * 16 + r % 16, 1.0, 0.0).astype(bf16)
        for t in range(NKT):
            kt = lax.dot_general(perm, aT[:, t * 128:(t + 1) * 128], NT, preferred_element_type=f32)
            k8_ref[t * 128:(t + 1) * 128, :] = kt.astype(jnp.int32).astype(jnp.int8)
        am = jnp.max(qs_ref[...] * ck[None], axis=1, keepdims=True)
        am = jnp.maximum(am, 2.0 ** -20)
        qs_ref[...] = ck[None] * (QMAX / am)
        sq_ref[...] = jnp.broadcast_to(am * (1.0 / (QMAX * QMAX)), (nblk, 8, TQ))
        for hp in range(NP):
            quant(0, hp)
        for cp in wcp:
            cp.wait()

    fast = flag_ref[0] > 0
    ist = jnp.minimum(i, nst - 1)
    hold = {}

    def rows(b):
        return pl.ds(pl.multiple_of((ist * NB + b) * TQ, TQ), TQ)

    def silu(y):
        u = 0.5 * y
        return u + u * jnp.tanh(u)

    def f1(b, c, half):
        ks = slice(half * HD, (half + 1) * HD)
        y = jnp.dot(xn_ref[rows(b), ks], w1_ref[ks, c * 128:(c + 1) * 128],
                    preferred_element_type=f32)
        if half == 0:
            hold[c] = y
        else:
            h_ref[:, c * 128:(c + 1) * 128] = silu(y + hold.pop(c)).astype(bf16)

    def f2(b, c, half):
        cs = slice(half * HD, (half + 1) * HD)
        y = jnp.dot(h_ref[:, c * 128:(c + 1) * 128], w2_ref[c * 128:(c + 1) * 128, cs],
                    preferred_element_type=f32)
        if c == 0:
            acc_ref[:, cs] = y + x_ref[rows(b), cs].astype(f32)
        else:
            acc_ref[:, cs] += y

    def op(b, n, half):
        cs = slice(half * HD, (half + 1) * HD)
        if half == 0:
            hold[("o", n)] = oT_ref[n * 128:(n + 1) * 128, :].T.astype(bf16)
            o = hold[("o", n)]
        else:
            o = hold.pop(("o", n))
        y = jnp.dot(o, wo_ref[n * 128:(n + 1) * 128, cs], preferred_element_type=f32)
        if n < 3:
            acc_ref[:, cs] += y
        else:
            res = (acc_ref[:, cs] + y).astype(o_ref.dtype)
            if b < NB - 1:
                stg_ref[b * TQ:(b + 1) * TQ, cs] = res
            else:
                o_ref[b * TQ:(b + 1) * TQ, cs] = res
                o_ref[0:b * TQ, cs] = stg_ref[0:b * TQ, cs]

    units = [(2 * g + half, 4 * t4)
             for g in range(NP // 2) for t4 in range(NKT // 4) for half in range(2)]
    nu = len(units)
    carry_a = [(NP - 2, NKT - 1)]
    carry_b = [(NP - 1, NKT - 4 + t) for t in range(4)]
    carry = carry_a + carry_b

    class Att:
        def __init__(self):
            self.pt, self.st, self.ls, self.cnt = {}, {}, {}, {}
            for n, hp in enumerate((NP - 2, NP - 1)):
                self.st[("c", hp)] = sc_ref[n]
                self.ls[("c", hp)] = lc_ref[n]
                self.cnt[("c", hp)] = NKT - sum(1 for c in carry if c[0] == hp)

        def pv(self, key, t):
            if isinstance(key, tuple):
                hp = key[1]
                p = pc_ref[carry.index((hp, t))]
            else:
                hp = key % NP
                p = self.pt.pop((key, t))
            o = jnp.dot(vT_ref[:, t * 128:(t + 1) * 128], p, preferred_element_type=f32)
            self.st[key] = o if key not in self.st else o + self.st[key]
            self.cnt[key] = self.cnt.get(key, 0) + 1
            if self.cnt[key] == NKT:
                l = jnp.sum(self.ls.pop(key), axis=0, keepdims=True)
                res = self.st.pop(key) * (1.0 / l)
                for u in range(2):
                    h = hp * 2 + u
                    oT_ref[h * DH:(h + 1) * DH, :] = res[:, u * TQ:(u + 1) * TQ] * cv_ref[...]

    @pl.when(jnp.logical_and(fast, i < nst))
    def _():
        A = Att()
        sqs = {}

        def qk(b, hp, t0):
            if b not in sqs:
                sqs[b] = jnp.concatenate([sq_ref[ist * NB + b]] * 2, axis=1)
            q8 = q8_ref[hp]
            wgt = jnp.concatenate([q8[0:32], q8[0:32], q8[32:64]], axis=0)
            s = jnp.dot(k8_ref[t0 * 128:(t0 + 4) * 128, 0:KD], wgt,
                        preferred_element_type=jnp.int32)
            p = jnp.exp2(s.astype(f32).reshape(64, 8, HW) * sqs[b][None])
            l = jnp.sum(p, axis=0)
            key = b * NP + hp
            A.ls[key] = l if t0 == 0 else A.ls[key] + l
            p = p.reshape(512, HW)
            for t in range(4):
                A.pt[(key, t0 + t)] = _rev16(p, t).astype(bf16)

        slot = []
        for b in range(NB):
            dense = []
            for c in range(NF + 2):
                if c < NF:
                    dense += [P_(f1, b, c, 0), P_(f1, b, c, 1)]
                if c >= 2:
                    dense += [P_(f2, b, c - 2, 0), P_(f2, b, c - 2, 1)]
            opq = [(3 + half, P_(op, (b - 1) % NB, 3, half)) for half in range(2)]
            opq += [(22 + 16 * n + half, P_(op, b, n, half)) for n in range(3) for half in range(2)]
            for j in range(nu):
                slot.append(opq.pop(0)[1] if opq and j >= opq[0][0] else dense.pop(0))
            assert not dense and not opq

        cQ, cP, cD = 256, 32, 128
        seqs = [[], []]
        tl = [[(("c", hp), t) for hp, t in carry_a], [(("c", hp), t) for hp, t in carry_b]]

        def phase(a, pat):
            for ch in pat:
                if ch == "D":
                    seqs[a].append((cD, "D", slot.pop(0)))
                else:
                    seqs[a].append((cP, "P", tl[a].pop(0)))

        phase(1, "PDPP")
        for jj in range(NB * nu):
            b, j = divmod(jj, nu)
            hp, t0 = units[j]
            seqs[j % 2].append((cQ, "Q", (b, hp, t0)))
            tl[j % 2] += [(b * NP + hp, t0 + t) for t in range(4)]
            phase(j % 2, "PPDPP" if jj < NB * nu - 1 else "P")
        busy = [0, 0]
        idx = [0, 0]
        while idx[0] < len(seqs[0]) or idx[1] < len(seqs[1]):
            first = idx[1] >= len(seqs[1]) or (idx[0] < len(seqs[0]) and busy[0] <= busy[1])
            a = 0 if first else 1
            cost, kind, pay = seqs[a][idx[a]]
            idx[a] += 1
            busy[a] += cost
            if kind == "Q":
                qk(*pay)
                if pay[2] == NKT - 4:
                    quant(jnp.minimum(ist * NB + pay[0] + 1, nblk - 1), pay[1])
            elif kind == "P":
                A.pv(*pay)
            else:
                pay()
        off = (NB - 1) * NP
        for n, (hp, t) in enumerate(carry):
            pc_ref[n] = A.pt.pop((off + hp, t))
        for n, hp in enumerate((NP - 2, NP - 1)):
            sc_ref[n] = A.st.pop(off + hp)
            lc_ref[n] = A.ls.pop(off + hp)

    @pl.when(jnp.logical_and(fast, i == nst))
    def _():
        A = Att()
        for hp, t in carry:
            A.pv(("c", hp), t)
        op(NB - 1, 3, 0)
        op(NB - 1, 3, 1)

    @pl.when(jnp.logical_not(fast))
    def _():
        o_ref[...] = stg_ref[...]

        @pl.when(i < nst)
        def _():
            kb = kvT_ref[0:DH, :].astype(bf16)

            def sub(b, carry_):
                def pair(hp, carry__):
                    qg = jnp.concatenate(
                        [qT_ref[ist * NB + b, pl.ds(pl.multiple_of((hp * 2 + u) * DH, DH), DH), :]
                         for u in range(2)], axis=1).astype(bf16)
                    s = lax.dot_general(kb, qg, TN, preferred_element_type=f32)
                    p = jnp.exp2(s - jnp.max(s, axis=0, keepdims=True))
                    l = jnp.sum(p, axis=0, keepdims=True)
                    o = jnp.dot(vT_ref[...], p.astype(bf16), preferred_element_type=f32)
                    res = o * (1.0 / l)
                    for u in range(2):
                        hr = pl.multiple_of((hp * 2 + u) * DH, DH)
                        oT_ref[pl.ds(hr, DH), :] = res[:, u * TQ:(u + 1) * TQ] * cv_ref[...]
                    return carry__
                lax.fori_loop(0, NP, pair, 0)
                hh = silu(jnp.dot(xn_ref[rows(b), :], w1_ref[...], preferred_element_type=f32))
                y = jnp.dot(hh.astype(bf16), w2_ref[...], preferred_element_type=f32)
                y = y + jnp.dot(oT_ref[...].T.astype(bf16), wo_ref[...], preferred_element_type=f32)
                y = y + x_ref[rows(b), :].astype(f32)
                stg_ref[pl.ds(pl.multiple_of(b * TQ, TQ), TQ), :] = y.astype(stg_ref.dtype)
                return carry_
            lax.fori_loop(0, NB, sub, 0)


@jax.jit
def pallas_parallel_sum__grouped_kv_mqa__dense_activation_silu__prompt_kernel(
    A_x: jax.Array,
    A_wq: jax.Array,
    A_wk: jax.Array,
    A_wv: jax.Array,
    A_wo: jax.Array,
    B_x: jax.Array,
    B_w1: jax.Array,
    B_w2: jax.Array,
):
    del B_x
    B, S, D = A_x.shape
    F = B_w1.shape[1]
    assert B == 1 and D == H * DH == 512 and S % (NB * TQ) == 0 and S % 512 == 0
    assert F % 128 == 0 and 4 * (F // 128) + 8 == NP * (S // 512)
    nblk = S // TQ
    hbm = pl.BlockSpec(memory_space=pl.ANY)
    out = pl.pallas_call(
        functools.partial(_kernel, S=S, D=D, F=F),
        grid=(nblk // NB + 1,),
        in_specs=[hbm] * 7,
        out_specs=pl.BlockSpec((NB * TQ, D), lambda i: (jnp.maximum(i - 1, 0), 0)),
        out_shape=jax.ShapeDtypeStruct((S, D), A_x.dtype),
        scratch_shapes=[
            pltpu.VMEM((S, D), bf16),
            pltpu.VMEM((D, D), bf16),
            pltpu.VMEM((D, D), bf16),
            pltpu.VMEM((D, F), bf16),
            pltpu.VMEM((F, D), bf16),
            pltpu.SemaphoreType.DMA((S // LC + 6,)),
            pltpu.VMEM((S, D), bf16),
            pltpu.VMEM((D + 2 * DH, D), bf16),
            pltpu.VMEM((2 * DH, S), f32),
            pltpu.VMEM((S, 128), jnp.int8),
            pltpu.VMEM((DH, S), bf16),
            pltpu.VMEM((DH, 128), f32),
            pltpu.VMEM((nblk, D, TQ), f32),
            pltpu.VMEM((NP, 64, HW), jnp.int8),
            pltpu.VMEM((nblk, 8, TQ), f32),
            pltpu.VMEM((nblk, DH, TQ), f32),
            pltpu.VMEM((D, TQ), f32),
            pltpu.VMEM((TQ, F), bf16),
            pltpu.VMEM((TQ, D), f32),
            pltpu.VMEM((5, 128, HW), bf16),
            pltpu.VMEM((2, DH, HW), f32),
            pltpu.VMEM((2, 8, HW), f32),
            pltpu.VMEM((NB * TQ, D), A_x.dtype),
            pltpu.SMEM((1,), jnp.int32),
        ],
        compiler_params=pltpu.CompilerParams(
            dimension_semantics=("arbitrary",), vmem_limit_bytes=64 * 1024 * 1024),
    )(A_x.reshape(S, D), A_wq, A_wk.T, A_wv.T, A_wo, B_w1, B_w2)
    return out.reshape(B, S, D)
```
